```python
import os as _os
_os.environ.setdefault("JAX_PLATFORMS", "cpu")
import jax
import jax.numpy as jnp

def _softmax(x, axis=-1):
    return jax.nn.softmax(x, axis=axis)
def _gelu(x):
    return jax.nn.gelu(x, approximate=True)
def _silu(x):
    return jax.nn.silu(x)
def _sigmoid(x):
    return jax.nn.sigmoid(x)
def _layernorm(x, axis=-1, eps=1e-5):
    m = jnp.mean(x, axis=axis, keepdims=True)
    v = jnp.var(x, axis=axis, keepdims=True)
    return (x - m) / jnp.sqrt(v + eps)
def _scatter_add(tgt, idx, src, axis=0):
    return tgt.at[idx].add(src)
def _segment_sum(src, seg, n):
    return jax.ops.segment_sum(src, seg, n)
class _Rng:
    def __init__(self, key):
        self._k = key
    def _next(self):
        self._k, sub = jax.random.split(self._k)
        return sub
    def normal(self, shape):
        return jax.random.normal(self._next(), shape, dtype=jnp.bfloat16)
    def randint(self, lo, hi, shape):
        return jax.random.randint(self._next(), shape, lo, hi, dtype=jnp.int32)
    def uniform(self, shape, lo=0.0, hi=1.0):
        return jax.random.uniform(self._next(), shape, jnp.bfloat16, lo, hi)
    def permutation(self, n):
        return jax.random.permutation(self._next(), n)


kernel_name = 'parallel_sum__ssm_conv_s4__mixer_channel_mlp__prompt'

def setup_inputs():
    _rng = _Rng(jax.random.key(int.from_bytes(__import__("os").urandom(4), "little")))
    _w = (lambda a: (lambda t: t.astype(jnp.bfloat16) if jnp.issubdtype(t.dtype, jnp.floating) else t)(jnp.asarray(a)))
    def _A_setup():
        B, L, D, N = 1, 2048, 512, 128
        A_re = -jnp.exp((lambda *s: _rng.normal(s) * 0.1)(D, N))
        A_im = jnp.pi * (lambda *s: _rng.normal(s) * 0.1)(D, N)
        B_re = (lambda *s: _rng.normal(s) * 0.1)(D, N)
        B_im = (lambda *s: _rng.normal(s) * 0.1)(D, N)
        C_re = (lambda *s: _rng.normal(s) * 0.1)(D, N)
        C_im = (lambda *s: _rng.normal(s) * 0.1)(D, N)
        log_dt = (lambda *s: _rng.normal(s) * 0.1)(D) * 0.5 - 4.0
        Dskip = (lambda *s: _rng.normal(s) * 0.05)(D)
        return {
            "u": _w((lambda *s: _rng.normal(s) * 0.05)(B, L, D)),
            "A_re": _w(A_re),
            "A_im": _w(A_im),
            "B_re": _w(B_re),
            "B_im": _w(B_im),
            "C_re": _w(C_re),
            "C_im": _w(C_im),
            "log_dt": _w(log_dt),
            "Dskip": _w(Dskip),
        }
    _A_in = _A_setup()

    def _B_setup():
        B, S, D, F = 1, 2048, 512, 1792
        return {
            "x": _w((lambda *s: _rng.normal(s) * 0.05)(B, S, D)),
            "w1": _w((lambda *s: _rng.normal(s) * 0.2)(D, F) * (D ** -0.5)),
            "b1": _w((lambda *s: _rng.normal(s) * 0.2)(F)),
            "w2": _w((lambda *s: _rng.normal(s) * 0.2)(F, D) * (F ** -0.5)),
            "b2": _w((lambda *s: _rng.normal(s) * 0.05)(D)),
        }
    _B_in = _B_setup()

    return {
        "A_u": _A_in["u"],
        "A_A_re": _A_in["A_re"],
        "A_A_im": _A_in["A_im"],
        "A_B_re": _A_in["B_re"],
        "A_B_im": _A_in["B_im"],
        "A_C_re": _A_in["C_re"],
        "A_C_im": _A_in["C_im"],
        "A_log_dt": _A_in["log_dt"],
        "A_Dskip": _A_in["Dskip"],
        "B_x": _B_in["x"],
        "B_w1": _B_in["w1"],
        "B_b1": _B_in["b1"],
        "B_w2": _B_in["w2"],
        "B_b2": _B_in["b2"],
    }

def reference(A_u, A_A_re, A_A_im, A_B_re, A_B_im, A_C_re, A_C_im, A_log_dt, A_Dskip, B_x, B_w1, B_b1, B_w2, B_b2):
    def _A_ref(u, A_re, A_im, B_re, B_im, C_re, C_im, log_dt, Dskip):
        Bsz, L, D = u.shape
        dt = jnp.exp(log_dt)[:, None]
        A = A_re + 1j * A_im
        Bc = B_re + 1j * B_im
        Cc = C_re + 1j * C_im
        logdA = dt * A
        dB = dt * Bc
        l = (lambda x, dt: x.astype(dt))(jnp.arange(L), A_re.dtype)
        P = jnp.exp(logdA[:, :, None] * l[None, None, :])
        K = jnp.einsum("dn,dnl,dn->dl", Cc, P, dB).real
        L2 = 2 * L
        Kp = jnp.pad(K, ((0, 0), (0, L)))
        up = (lambda x, *d: x.transpose(*d))(u, 0, 2, 1)
        up = jnp.pad(up, ((0, 0), (0, 0), (0, L)))
        Kf = (lambda x, axes=(-2,-1): jnp.fft.rfft2(x.astype(jnp.float32), axes=axes))(Kp[:, None, :], axes=(-2, -1))
        Uf = (lambda x, axes=(-2,-1): jnp.fft.rfft2(x.astype(jnp.float32), axes=axes))(up[:, :, None, :], axes=(-2, -1))
        Yf = Uf * Kf[None, :, :, :]
        y = (lambda x, s, axes=(-2,-1): jnp.fft.irfft2(x, s=s, axes=axes).astype(jnp.bfloat16))(Yf, (1, L2), axes=(-2, -1))[:, :, 0, :L]
        y = (lambda x, *d: x.transpose(*d))(y, 0, 2, 1) + u * Dskip[None, None, :]
        return y

    def _B_ref(x, w1, b1, w2, b2):
        y = _layernorm(x, axis=-1)
        h = _gelu(jnp.einsum("bsd,df->bsf", y, w1) + b1)
        return jnp.einsum("bsf,fd->bsd", h, w2) + b2

    x = A_u
    xn = _layernorm(x, axis=-1)
    return x + _A_ref(xn, A_A_re, A_A_im, A_B_re, A_B_im, A_C_re, A_C_im, A_log_dt, A_Dskip) + _B_ref(xn, B_w1, B_b1, B_w2, B_b2)
```

```python
import functools

import jax
import jax.experimental.pallas as pl
import jax.experimental.pallas.tpu as pltpu
import jax.numpy as jnp
import ml_dtypes
import numpy as np
from jax import lax

bf16 = jnp.bfloat16
f32 = jnp.float32

T = 128
NB = 16
D_MODEL = 512
KDEP = 5

_L1 = [
    [j for j in range(8)],
    [128 + j for j in range(8)],
    [256 + o + 128 * h for h in range(2) for o in (0, 2, 4, 6)],
    [512 + o + 128 * h for h in range(4) for o in (0, 4)],
    [1024 + 128 * h for h in range(8)],
]
_TILE_BLOCKS = [(0,), (1,), (2, 3), (4, 5, 6, 7), (8, 9, 10, 11, 12, 13, 14, 15)]
_EXTRA = {3: 512, 7: 1024, 15: 2048}


@functools.lru_cache(maxsize=None)
def _constants():
    L = T * NB
    r_of_l = np.arange(L, dtype=np.float32).astype(ml_dtypes.bfloat16).astype(np.float32).astype(np.int64)
    where = {}
    for t, l1s in enumerate(_L1):
        for j, l1 in enumerate(l1s):
            for l2 in range(16):
                where[l1 + 8 * l2] = (t, (8 * l2 + 7 + j) % 128)
    th = 2 * np.pi * (np.arange(128) + 0.5) / 256

    def dft_cols(pos):
        ang = th[:, None] * np.asarray(pos)[None, :]
        return np.concatenate([np.cos(ang), -np.sin(ang)], 0)

    rows = []
    gx = np.zeros((256, 8))
    xi = 0
    for t, blocks in enumerate(_TILE_BLOCKS):
        for i in blocks:
            g = np.zeros((256, 128))
            for p in range(128):
                r = int(r_of_l[128 * i + p])
                if i in _EXTRA and r == _EXTRA[i]:
                    gx[:, xi] += dft_cols([p])[:, 0]
                else:
                    tt, lane = where[r]
                    assert tt == t
                    g[:, lane] += dft_cols([p])[:, 0]
            if i in _EXTRA:
                xi += 1
            rows.append(g)
    sel = np.zeros((3, 16, 128))
    sel[0, 0, where[512][1]] = 1.0
    sel[1, 0, where[1024][1]] = 1.0
    sel[2, 0, 0] = 1.0
    fwd = dft_cols(np.arange(128))
    inv = fwd.T / 128

    def cast(a):
        return np.asarray(a, np.float32).astype(ml_dtypes.bfloat16)

    return (cast(fwd), cast(inv), cast(np.concatenate(rows, 0)), cast(sel.reshape(48, 128)),
            np.asarray(gx, np.float32))


def _cmul(a, b):
    return (a[0] * b[0] - a[1] * b[1], a[0] * b[1] + a[1] * b[0])


def _csq(a):
    t = a[0] * a[1]
    return (a[0] * a[0] - a[1] * a[1], t + t)


def _ln(x):
    m = jnp.mean(x, axis=-1, keepdims=True)
    xc = x - m
    v = jnp.mean(xc * xc, axis=-1, keepdims=True)
    return xc * lax.rsqrt(v + 1e-5)


def _gelu(x):
    return 0.5 * x * (1.0 + jnp.tanh(0.7978845608028654 * (x + 0.044715 * (x * x * x))))


def _nt(a, b):
    return lax.dot_general(a, b, (((1,), (1,)), ((), ())), preferred_element_type=f32)


def _flip8(x):
    s = lax.broadcasted_iota(jnp.int32, (8, 128), 0)
    x = pltpu.roll(x, 4, 0)
    x = jnp.where((s & 2) == 0, pltpu.roll(x, 6, 0), pltpu.roll(x, 2, 0))
    x = jnp.where((s & 1) == 0, pltpu.roll(x, 7, 0), pltpu.roll(x, 1, 0))
    return x


def _cis(x):
    q = jnp.floor(x * 0.6366197723675814 + 0.5)
    r = x - q * 1.5703125
    r = r - q * 4.837512969970703125e-4
    r = r - q * 7.54978995489188216e-8
    z = r * r
    s = r + r * z * (-1.6666654611e-1 + z * (8.3321608736e-3 + z * -1.9515295891e-4))
    c = (1.0 - 0.5 * z) + z * z * (4.166664568298827e-2 + z * (-1.388731625493765e-3 + z * 2.443315711809948e-5))
    qi = q.astype(jnp.int32)
    swap = (qi & 1) != 0
    cs = jnp.where(swap, s, c)
    sn = jnp.where(swap, c, s)
    sn = jnp.where((qi & 2) != 0, -sn, sn)
    cs = jnp.where(((qi + 1) & 2) != 0, -cs, cs)
    return cs, sn


def _taps_group(r, prm, dt_ref, kt_ref, dep):
    are, aim, bre, bim, cre, cim = [ref[r, :].astype(f32) for ref in prm]
    dt = dt_ref[r, :]
    if dep is not None:
        dt = jnp.where(dep[0], dep[1], dt)
    xr = dt * are
    xi = dt * aim
    w = _cmul((cre, cim), (dt * bre, dt * bim))
    e1 = jnp.exp(xr)
    c_, s_ = _cis(xi)
    a1 = (e1 * c_, e1 * s_)
    a8 = _csq(_csq(_csq(a1)))
    a128 = _csq(_csq(_csq(_csq(a8))))
    a256 = _csq(a128)
    a512 = _csq(a256)
    a1024 = _csq(a512)
    a8c = (_flip8(a8[0]), -_flip8(a8[1]))
    v = [(jnp.ones_like(xr), jnp.zeros_like(xr)), a8c]
    for l2 in range(2, 16):
        v.append(_csq(v[l2 // 2]) if l2 % 2 == 0 else _cmul(v[l2 - 1], a8c))
    vre = jnp.concatenate([p[0] for p in v], axis=0)
    vim = jnp.concatenate([p[1] for p in v], axis=0)
    vt = jnp.concatenate([vre, vim], axis=1).astype(bf16)
    c0 = [w]
    for _ in range(1, 8):
        c0.append(_cmul(c0[-1], a1))
    c1 = [_cmul(c, a128) for c in c0]
    c2a = [_cmul(c0[o], a256) for o in (0, 2, 4, 6)]
    c2 = c2a + [_cmul(c, a128) for c in c2a]
    c3 = [_cmul(c0[0], a512), _cmul(c0[4], a512)]
    for _ in range(1, 4):
        c3 += [_cmul(c3[-2], a128), _cmul(c3[-1], a128)]
    c4 = [_cmul(c0[0], a1024)]
    for _ in range(1, 8):
        c4.append(_cmul(c4[-1], a128))
    k2048 = jnp.sum(c4[-1][0] * a128[0] - c4[-1][1] * a128[1], axis=1, keepdims=True)
    cs = c0 + c1 + c2 + c3 + c4
    lhs = jnp.concatenate([jnp.concatenate([p[0] for p in cs], axis=0),
                           jnp.concatenate([p[1] for p in cs], axis=0)], axis=1).astype(bf16)
    out = _nt(lhs, vt)
    lane8 = lax.broadcasted_iota(jnp.int32, (8, 128), 1) & 7
    kt_ref[5, r, :] = jnp.broadcast_to(k2048, (8, 128))
    for t in range(5):
        for j in range(8):
            xj = out[(t * 8 + j) * 8:(t * 8 + j) * 8 + 8, :]
            xj = pltpu.roll(xj, j, 1, stride=1, stride_axis=0)
            pltpu.store(kt_ref.at[t, r, :], xj, mask=(lane8 == (j + 7) % 8))
    return out[0:8, :]


def _kernel(x_hbm, are_ref, aim_ref, bre_ref, bim_ref, cre_ref, cim_ref, logdt_ref, dskip_ref, z_ref,
            w1_hbm, b1_ref, w2_hbm, b2_ref, f_ref, finv_ref, sel_ref, gx_ref, g_hbm, o_hbm,
            x_ref, w1_ref, w2_ref, g_ref, o_ref, dt_ref, kt_ref, kf_ref, u_ref, in_sems, out_sems):
    cp_g = pltpu.make_async_copy(g_hbm, g_ref, in_sems.at[0])
    cp_x = pltpu.make_async_copy(x_hbm, x_ref, in_sems.at[1])
    cp_w1 = pltpu.make_async_copy(w1_hbm, w1_ref, in_sems.at[2])
    cp_w2 = pltpu.make_async_copy(w2_hbm, w2_ref, in_sems.at[3])
    cp_g.start()
    cp_x.start()
    cp_w1.start()
    cp_w2.start()

    dtrow = jnp.exp(logdt_ref[...].astype(f32).reshape(1, D_MODEL)).astype(bf16).astype(f32)
    dt_ref[...] = jnp.broadcast_to(dtrow, (128, D_MODEL)).T
    prm = [are_ref, aim_ref, bre_ref, bim_ref, cre_ref, cim_ref]
    never = jnp.full((8, 128), z_ref[0], jnp.int32) != 0
    outs = []
    for q in range(D_MODEL // 8):
        dep = (never, outs[q - KDEP]) if q >= KDEP else None
        outs.append(_taps_group(pl.ds(q * 8, 8), prm, dt_ref, kt_ref, dep))

    cp_g.wait()
    ktb = [kt_ref[t].astype(bf16) for t in range(6)]
    extra_row = [_nt(sel_ref[0:16, :], ktb[3])[0:1], _nt(sel_ref[16:32, :], ktb[4])[0:1],
                 _nt(sel_ref[32:48, :], ktb[5])[0:1]]
    gx = gx_ref[...]
    sgn = 1.0 - 2.0 * (lax.broadcasted_iota(jnp.int32, (128, D_MODEL), 0) % 2).astype(f32)
    prev = None
    xi = 0
    for t, blocks in enumerate(_TILE_BLOCKS):
        for i in blocks:
            acc = _nt(g_ref[pl.ds(i * 256, 256), :], ktb[t])
            if i in _EXTRA:
                acc = acc + jnp.broadcast_to(gx[:, xi:xi + 1], (256, D_MODEL)) * extra_row[xi]
                xi += 1
            re, im = acc[:128], acc[128:]
            if prev is not None:
                kf_ref[i, :128, :] = re - sgn * prev[1]
                kf_ref[i, 128:, :] = im + sgn * prev[0]
            else:
                kf_ref[i] = acc
            prev = (re, im)

    cp_x.wait()
    cp_w1.wait()
    cp_w2.wait()
    dskip = dskip_ref[...].astype(f32).reshape(1, -1)
    b1 = b1_ref[...].astype(f32).reshape(1, -1)
    b2 = b2_ref[...].astype(f32).reshape(1, -1)

    def out_copy(m):
        rows = pl.ds(m * T, T)
        return pltpu.make_async_copy(o_ref.at[rows, :], o_hbm.at[rows, :], out_sems.at[m])

    for m in range(NB):
        rows = pl.ds(m * T, T)
        x = x_ref[rows, :].astype(f32)
        xn = _ln(x).astype(bf16)
        xnf = xn.astype(f32)
        u_ref[m] = jnp.dot(f_ref[...], xn, preferred_element_type=f32)
        ys = []
        for c in range(D_MODEL // 128):
            cs = pl.ds(c * 128, 128)
            yr = yi = None
            for j in range(m + 1):
                ur = u_ref[j, 0:128, cs]
                ui = u_ref[j, 128:256, cs]
                kr = kf_ref[m - j, 0:128, cs]
                ki = kf_ref[m - j, 128:256, cs]
                pr = ur * kr - ui * ki
                pi = ur * ki + ui * kr
                yr = pr if yr is None else yr + pr
                yi = pi if yi is None else yi + pi
            ys.append(jnp.concatenate([yr, yi], axis=0).astype(bf16))
        y = jnp.dot(finv_ref[...], jnp.concatenate(ys, axis=1), preferred_element_type=f32)
        y2 = _ln(xnf).astype(bf16)
        h = jnp.dot(y2, w1_ref[...], preferred_element_type=f32) + b1
        h = _gelu(h).astype(bf16)
        o = jnp.dot(h, w2_ref[...], preferred_element_type=f32) + b2
        o_ref[rows, :] = (x + (y + xnf * dskip) + o).astype(bf16)
        out_copy(m).start()
    for m in range(NB):
        out_copy(m).wait()


@jax.jit
def pallas_parallel_sum__ssm_conv_s4__mixer_channel_mlp__prompt_kernel(
    A_u: jax.Array,
    A_A_re: jax.Array,
    A_A_im: jax.Array,
    A_B_re: jax.Array,
    A_B_im: jax.Array,
    A_C_re: jax.Array,
    A_C_im: jax.Array,
    A_log_dt: jax.Array,
    A_Dskip: jax.Array,
    B_x: jax.Array,
    B_w1: jax.Array,
    B_b1: jax.Array,
    B_w2: jax.Array,
    B_b2: jax.Array,
):
    del B_x
    B, L, D = A_u.shape
    F = B_w1.shape[1]
    assert (B, L, D) == (1, T * NB, D_MODEL) and A_A_re.shape == (D, 128)
    fwd, inv, g, sel, gx = _constants()
    hbm = pl.BlockSpec(memory_space=pl.ANY)
    vm = pl.BlockSpec(memory_space=pltpu.VMEM)
    sm = pl.BlockSpec(memory_space=pltpu.SMEM)
    out = pl.pallas_call(
        _kernel,
        out_shape=jax.ShapeDtypeStruct((L, D), bf16),
        in_specs=[hbm] + [vm] * 8 + [sm, hbm, vm, hbm, vm, vm, vm, vm, vm, hbm],
        out_specs=hbm,
        scratch_shapes=[
            pltpu.VMEM((L, D), bf16),
            pltpu.VMEM((D, F), bf16),
            pltpu.VMEM((F, D), bf16),
            pltpu.VMEM(g.shape, bf16),
            pltpu.VMEM((L, D), bf16),
            pltpu.VMEM((D, 128), f32),
            pltpu.VMEM((6, D, 128), f32),
            pltpu.VMEM((NB, 256, D), f32),
            pltpu.VMEM((NB, 256, D), f32),
            pltpu.SemaphoreType.DMA((4,)),
            pltpu.SemaphoreType.DMA((NB,)),
        ],
        compiler_params=pltpu.CompilerParams(vmem_limit_bytes=100 * 1024 * 1024),
    )(A_u.astype(bf16).reshape(L, D), A_A_re, A_A_im, A_B_re, A_B_im, A_C_re, A_C_im, A_log_dt, A_Dskip,
      jnp.asarray(np.zeros((1,), np.int32)), B_w1, B_b1, B_w2, B_b2,
      jnp.asarray(fwd), jnp.asarray(inv), jnp.asarray(sel), jnp.asarray(gx), jnp.asarray(g))
    return out.reshape(B, L, D).astype(A_u.dtype)
```

```python
import functools

import jax
import jax.experimental.pallas as pl
import jax.experimental.pallas.tpu as pltpu
import jax.numpy as jnp
import ml_dtypes
import numpy as np
from jax import lax

bf16 = jnp.bfloat16
f32 = jnp.float32

T = 128
NB = 16
D_MODEL = 512
KDEP = 5

_L1 = [
    [j for j in range(8)],
    [128 + j for j in range(8)],
    [256 + o + 128 * h for h in range(2) for o in (0, 2, 4, 6)],
    [512 + o + 128 * h for h in range(4) for o in (0, 4)],
    [1024 + 128 * h for h in range(8)],
]
_TILE_BLOCKS = [(0,), (1,), (2, 3), (4, 5, 6, 7), (8, 9, 10, 11, 12, 13, 14, 15)]
_EXTRA = {3: 512, 7: 1024, 15: 2048}


@functools.lru_cache(maxsize=None)
def _constants():
    L = T * NB
    r_of_l = np.arange(L, dtype=np.float32).astype(ml_dtypes.bfloat16).astype(np.float32).astype(np.int64)
    where = {}
    for t, l1s in enumerate(_L1):
        for j, l1 in enumerate(l1s):
            for l2 in range(16):
                where[l1 + 8 * l2] = (t, (8 * l2 + 7 + j) % 128)
    th = 2 * np.pi * (np.arange(128) + 0.5) / 256

    def dft_cols(pos):
        ang = th[:, None] * np.asarray(pos)[None, :]
        return np.concatenate([np.cos(ang), -np.sin(ang)], 0)

    rows = []
    gx = np.zeros((256, 128))
    xi = 0
    for t, blocks in enumerate(_TILE_BLOCKS):
        for i in blocks:
            g = np.zeros((256, 128))
            for p in range(128):
                r = int(r_of_l[128 * i + p])
                if i in _EXTRA and r == _EXTRA[i]:
                    gx[:, xi] += dft_cols([p])[:, 0]
                else:
                    tt, lane = where[r]
                    assert tt == t
                    g[:, lane] += dft_cols([p])[:, 0]
            if i in _EXTRA:
                xi += 1
            rows.append(g)
    sel = np.zeros((3, 16, 128))
    sel[0, 0, where[512][1]] = 1.0
    sel[1, 0, where[1024][1]] = 1.0
    sel[2, 0, 0] = 1.0
    fwd = dft_cols(np.arange(128))
    inv = fwd.T / 128

    packed = np.concatenate(rows + [fwd, inv[:, :128], inv[:, 128:], gx, sel.reshape(48, 128)], 0)
    return np.asarray(packed, np.float32).astype(ml_dtypes.bfloat16)


def _cmul(a, b):
    return (a[0] * b[0] - a[1] * b[1], a[0] * b[1] + a[1] * b[0])


def _csq(a):
    t = a[0] * a[1]
    return (a[0] * a[0] - a[1] * a[1], t + t)


def _ln(x):
    m = jnp.mean(x, axis=-1, keepdims=True)
    xc = x - m
    v = jnp.mean(xc * xc, axis=-1, keepdims=True)
    return xc * lax.rsqrt(v + 1e-5)


def _gelu2(x):
    inner = x * (0.7978845608028654 + (0.7978845608028654 * 0.044715) * (x * x))
    return x + x * jnp.tanh(inner)


def _nt(a, b):
    return lax.dot_general(a, b, (((1,), (1,)), ((), ())), preferred_element_type=f32)


def _flip8(x):
    s = lax.broadcasted_iota(jnp.int32, (8, 128), 0)
    x = pltpu.roll(x, 4, 0)
    x = jnp.where((s & 2) == 0, pltpu.roll(x, 6, 0), pltpu.roll(x, 2, 0))
    x = jnp.where((s & 1) == 0, pltpu.roll(x, 7, 0), pltpu.roll(x, 1, 0))
    return x


def _cis(x):
    q = jnp.floor(x * 0.6366197723675814 + 0.5)
    r = x - q * 1.5703125
    r = r - q * 4.837512969970703125e-4
    r = r - q * 7.54978995489188216e-8
    z = r * r
    s = r + r * z * (-1.6666654611e-1 + z * (8.3321608736e-3 + z * -1.9515295891e-4))
    c = (1.0 - 0.5 * z) + z * z * (4.166664568298827e-2 + z * (-1.388731625493765e-3 + z * 2.443315711809948e-5))
    qi = q.astype(jnp.int32)
    swap = (qi & 1) != 0
    cs = jnp.where(swap, s, c)
    sn = jnp.where(swap, c, s)
    sn = jnp.where((qi & 2) != 0, -sn, sn)
    cs = jnp.where(((qi + 1) & 2) != 0, -cs, cs)
    return cs, sn


def _taps_group(r, prm, dt_ref, kt_ref, dep):
    are, aim, bre, bim, cre, cim = [ref[r, :].astype(f32) for ref in prm]
    dt = dt_ref[r, :]
    if dep is not None:
        dt = jnp.where(dep[0], dep[1], dt)
    xr = dt * are
    xi = dt * aim
    w = _cmul((cre, cim), (dt * bre, dt * bim))
    e1 = jnp.exp(xr)
    c_, s_ = _cis(xi)
    a1 = (e1 * c_, e1 * s_)
    a8 = _csq(_csq(_csq(a1)))
    a128 = _csq(_csq(_csq(_csq(a8))))
    a256 = _csq(a128)
    a512 = _csq(a256)
    a1024 = _csq(a512)
    a8c = (_flip8(a8[0]), -_flip8(a8[1]))
    v = [(jnp.ones_like(xr), jnp.zeros_like(xr)), a8c]
    for l2 in range(2, 16):
        v.append(_csq(v[l2 // 2]) if l2 % 2 == 0 else _cmul(v[l2 - 1], a8c))
    vre = jnp.concatenate([p[0] for p in v], axis=0)
    vim = jnp.concatenate([p[1] for p in v], axis=0)
    vt = jnp.concatenate([vre, vim], axis=1).astype(bf16)
    c0 = [w]
    for _ in range(1, 8):
        c0.append(_cmul(c0[-1], a1))
    c1 = [_cmul(c, a128) for c in c0]
    c2a = [_cmul(c0[o], a256) for o in (0, 2, 4, 6)]
    c2 = c2a + [_cmul(c, a128) for c in c2a]
    c3 = [_cmul(c0[0], a512), _cmul(c0[4], a512)]
    for _ in range(1, 4):
        c3 += [_cmul(c3[-2], a128), _cmul(c3[-1], a128)]
    c4 = [_cmul(c0[0], a1024)]
    for _ in range(1, 8):
        c4.append(_cmul(c4[-1], a128))
    k2048 = jnp.sum(c4[-1][0] * a128[0] - c4[-1][1] * a128[1], axis=1, keepdims=True)
    cs = c0 + c1 + c2 + c3 + c4
    lhs = jnp.concatenate([jnp.concatenate([p[0] for p in cs], axis=0),
                           jnp.concatenate([p[1] for p in cs], axis=0)], axis=1).astype(bf16)
    out = _nt(lhs, vt)
    lane8 = lax.broadcasted_iota(jnp.int32, (8, 128), 1) & 7
    kt_ref[5, r, :] = jnp.broadcast_to(k2048, (8, 128))
    for t in range(5):
        for j in range(8):
            xj = out[(t * 8 + j) * 8:(t * 8 + j) * 8 + 8, :]
            xj = pltpu.roll(xj, j, 1, stride=1, stride_axis=0)
            pltpu.store(kt_ref.at[t, r, :], xj, mask=(lane8 == (j + 7) % 8))
    return out[0:8, :]


def _kernel(x_hbm, are_ref, aim_ref, bre_ref, bim_ref, cre_ref, cim_ref, logdt_ref, dskip_ref, z_ref,
            w1_hbm, b1_ref, w2_hbm, b2_ref, g_hbm, o_hbm,
            x_ref, w1_ref, w2_ref, w1p_ref, w2p_ref, g_ref, o_ref, dt_ref, kt_ref, kf_ref, u_ref, in_sems, out_sems):
    cp_g = pltpu.make_async_copy(g_hbm, g_ref, in_sems.at[0])
    cp_x = pltpu.make_async_copy(x_hbm, x_ref, in_sems.at[1])
    cp_w1 = pltpu.make_async_copy(w1_hbm, w1_ref, in_sems.at[2])
    cp_w2 = pltpu.make_async_copy(w2_hbm, w2_ref, in_sems.at[3])
    f_ref = g_ref.at[pl.ds(4096, 256), :]
    finv_ref = g_ref.at[pl.ds(4352, 256), :]
    gx_ref = g_ref.at[pl.ds(4608, 256), :]
    sel_ref = g_ref.at[pl.ds(4864, 48), :]
    cp_g.start()
    cp_x.start()
    cp_w1.start()
    cp_w2.start()

    dtrow = jnp.exp(logdt_ref[...].astype(f32).reshape(1, D_MODEL)).astype(bf16).astype(f32)
    dt_ref[...] = jnp.broadcast_to(dtrow, (128, D_MODEL)).T
    prm = [are_ref, aim_ref, bre_ref, bim_ref, cre_ref, cim_ref]
    never = jnp.full((8, 128), z_ref[0], jnp.int32) != 0
    outs = []
    for q in range(D_MODEL // 8):
        dep = (never, outs[q - KDEP]) if q >= KDEP else None
        outs.append(_taps_group(pl.ds(q * 8, 8), prm, dt_ref, kt_ref, dep))

    cp_g.wait()
    ktb = [kt_ref[t].astype(bf16) for t in range(6)]
    extra_row = [_nt(sel_ref[0:16, :], ktb[3])[0:1], _nt(sel_ref[16:32, :], ktb[4])[0:1],
                 _nt(sel_ref[32:48, :], ktb[5])[0:1]]
    gx = gx_ref[...].astype(f32)
    sgn = 1.0 - 2.0 * (lax.broadcasted_iota(jnp.int32, (128, D_MODEL), 0) % 2).astype(f32)
    prev = None
    xi = 0
    for t, blocks in enumerate(_TILE_BLOCKS):
        for i in blocks:
            acc = _nt(g_ref[pl.ds(i * 256, 256), :], ktb[t])
            if i in _EXTRA:
                acc = acc + jnp.broadcast_to(gx[:, xi:xi + 1], (256, D_MODEL)) * extra_row[xi]
                xi += 1
            re, im = acc[:128], acc[128:]
            if prev is not None:
                kf_ref[i, :128, :] = re - sgn * prev[1]
                kf_ref[i, 128:, :] = im + sgn * prev[0]
            else:
                kf_ref[i] = acc
            prev = (re, im)

    cp_x.wait()
    cp_w1.wait()
    cp_w2.wait()
    finv = jnp.concatenate([finv_ref[0:128, :].astype(f32), finv_ref[128:256, :].astype(f32)], axis=1).astype(bf16)
    dskip = dskip_ref[...].astype(f32).reshape(1, -1)
    b1 = b1_ref[...].astype(f32).reshape(1, -1)
    b2 = b2_ref[...].astype(f32).reshape(1, -1)

    def out_copy(m):
        rows = pl.ds(m * T, T)
        return pltpu.make_async_copy(o_ref.at[rows, :], o_hbm.at[rows, :], out_sems.at[m])

    for m in range(NB):
        rows = pl.ds(m * T, T)
        xs = [x_ref[pl.ds(m * T + r0, 32), :].astype(f32) for r0 in range(0, T, 32)]
        xnfs = [_ln(v).astype(bf16).astype(f32) for v in xs]
        x = jnp.concatenate(xs, axis=0)
        xnf = jnp.concatenate(xnfs, axis=0)
        xn = xnf.astype(bf16)
        u_ref[m] = jnp.dot(f_ref[...], xn, preferred_element_type=f32)
        ys = []
        for c in range(D_MODEL // 128):
            cs = pl.ds(c * 128, 128)
            yr = yi = None
            for j in range(m + 1):
                ur = u_ref[j, 0:128, cs]
                ui = u_ref[j, 128:256, cs]
                kr = kf_ref[m - j, 0:128, cs]
                ki = kf_ref[m - j, 128:256, cs]
                pr = ur * kr - ui * ki
                pi = ur * ki + ui * kr
                yr = pr if yr is None else yr + pr
                yi = pi if yi is None else yi + pi
            ys.append(jnp.concatenate([yr, yi], axis=0).astype(bf16))
        y = jnp.dot(finv, jnp.concatenate(ys, axis=1), preferred_element_type=f32)
        y2 = jnp.concatenate([_ln(v) for v in xnfs], axis=0).astype(bf16)
        if m == 0:
            w1 = w1_ref[...]
            w2 = w2_ref[...]
            w1p_ref[...] = pltpu.bitcast(w1, jnp.uint32)
            w2p_ref[...] = pltpu.bitcast(w2, jnp.uint32)
        else:
            w1 = pltpu.bitcast(w1p_ref[...], bf16)
            w2 = pltpu.bitcast(w2p_ref[...], bf16)
        h = jnp.dot(y2, w1, preferred_element_type=f32) + b1
        h = _gelu2(h).astype(bf16)
        o = 0.5 * jnp.dot(h, w2, preferred_element_type=f32) + b2
        o_ref[rows, :] = (x + (y + xnf * dskip) + o).astype(bf16)
        out_copy(m).start()
    for m in range(NB):
        out_copy(m).wait()


@jax.jit
def pallas_parallel_sum__ssm_conv_s4__mixer_channel_mlp__prompt_kernel(
    A_u: jax.Array,
    A_A_re: jax.Array,
    A_A_im: jax.Array,
    A_B_re: jax.Array,
    A_B_im: jax.Array,
    A_C_re: jax.Array,
    A_C_im: jax.Array,
    A_log_dt: jax.Array,
    A_Dskip: jax.Array,
    B_x: jax.Array,
    B_w1: jax.Array,
    B_b1: jax.Array,
    B_w2: jax.Array,
    B_b2: jax.Array,
):
    del B_x
    B, L, D = A_u.shape
    F = B_w1.shape[1]
    assert (B, L, D) == (1, T * NB, D_MODEL) and A_A_re.shape == (D, 128)
    g = _constants()
    hbm = pl.BlockSpec(memory_space=pl.ANY)
    vm = pl.BlockSpec(memory_space=pltpu.VMEM)
    sm = pl.BlockSpec(memory_space=pltpu.SMEM)
    out = pl.pallas_call(
        _kernel,
        out_shape=jax.ShapeDtypeStruct((L, D), bf16),
        in_specs=[hbm] + [vm] * 8 + [sm, hbm, vm, hbm, vm, hbm],
        out_specs=hbm,
        scratch_shapes=[
            pltpu.VMEM((L, D), bf16),
            pltpu.VMEM((D, F), bf16),
            pltpu.VMEM((F, D), bf16),
            pltpu.VMEM((D // 2, F), jnp.uint32),
            pltpu.VMEM((F // 2, D), jnp.uint32),
            pltpu.VMEM(g.shape, bf16),
            pltpu.VMEM((L, D), bf16),
            pltpu.VMEM((D, 128), f32),
            pltpu.VMEM((6, D, 128), f32),
            pltpu.VMEM((NB, 256, D), f32),
            pltpu.VMEM((NB, 256, D), f32),
            pltpu.SemaphoreType.DMA((4,)),
            pltpu.SemaphoreType.DMA((NB,)),
        ],
        compiler_params=pltpu.CompilerParams(vmem_limit_bytes=100 * 1024 * 1024),
    )(A_u.astype(bf16).reshape(L, D), A_A_re, A_A_im, A_B_re, A_B_im, A_C_re, A_C_im, A_log_dt, A_Dskip,
      jnp.asarray(np.zeros((1,), np.int32)), B_w1.astype(bf16), B_b1, B_w2.astype(bf16), B_b2,
      jnp.asarray(g))
    return out.reshape(B, L, D).astype(A_u.dtype)
```
